```python
import jax
import jax.numpy as jnp

def _softmax(x, axis=-1):
    return jax.nn.softmax(x, axis=axis)
def _gelu(x):
    return jax.nn.gelu(x, approximate=True)
def _silu(x):
    return jax.nn.silu(x)
def _sigmoid(x):
    return jax.nn.sigmoid(x)
def _layernorm(x, axis=-1, eps=1e-5):
    m = jnp.mean(x, axis=axis, keepdims=True)
    v = jnp.var(x, axis=axis, keepdims=True)
    return (x - m) / jnp.sqrt(v + eps)
def _scatter_add(tgt, idx, src, axis=0):
    return tgt.at[idx].add(src)
def _segment_sum(src, seg, n):
    return jax.ops.segment_sum(src, seg, n)
class _Rng:
    def __init__(self, key):
        self._k = key
    def _next(self):
        self._k, sub = jax.random.split(self._k)
        return sub
    def normal(self, shape):
        return jax.random.normal(self._next(), shape, dtype=jnp.bfloat16)
    def randint(self, lo, hi, shape):
        return jax.random.randint(self._next(), shape, lo, hi, dtype=jnp.int32)
    def uniform(self, shape, lo=0.0, hi=1.0):
        return jax.random.uniform(self._next(), shape, jnp.bfloat16, lo, hi)
    def permutation(self, n):
        return jax.random.permutation(self._next(), n)


kernel_name = 'sequential_preLN__sliding_block_cached__glu_gated_swiglu__decode'

def setup_inputs():
    _rng = _Rng(jax.random.key(int.from_bytes(__import__("os").urandom(4), "little")))
    _w = (lambda a: (lambda t: t.astype(jnp.bfloat16) if jnp.issubdtype(t.dtype, jnp.floating) else t)(jnp.asarray(a)))
    def _A_setup():
        B, Sq, D = 1, 1, 640
        Hq, Hkv, Sk, Dh = 32, 32, 32768, 192
        assert Hq % Hkv == 0, (Hq, Hkv)
        return {
            "x": _w((lambda *s: _rng.normal(s) * 0.05)(B, Sq, D)),
            "k_cache": _w((lambda *s: _rng.normal(s) * 0.05)(B, Hkv, Sk, Dh)),
            "v_cache": _w((lambda *s: _rng.normal(s) * 0.05)(B, Hkv, Sk, Dh)),
            "wq": _w((lambda *s: _rng.normal(s) * 0.05)(D, Hq * Dh) * (D ** -0.5)),
            "wo": _w((lambda *s: _rng.normal(s) * 0.05)(Hq * Dh, D) * ((Hq * Dh) ** -0.5)),
        }
    _A_in = _A_setup()

    def _B_setup():
        B, S, D, F = 1, 1, 640, 1536
        return {
            "x": _w((lambda *s: _rng.normal(s) * 0.05)(B, S, D)),
            "w1": _w((lambda *s: _rng.normal(s) * 0.05)(D, F) * (2.0 / D) ** 0.5),
            "w3": _w((lambda *s: _rng.normal(s) * 0.05)(D, F) * (2.0 / D) ** 0.5),
            "w2": _w((lambda *s: _rng.normal(s) * 0.05)(F, D) * (2.0 / F) ** 0.5),
        }
    _B_in = _B_setup()

    return {
        "A_x": _A_in["x"],
        "A_k_cache": _A_in["k_cache"],
        "A_v_cache": _A_in["v_cache"],
        "A_wq": _A_in["wq"],
        "A_wo": _A_in["wo"],
        "B_x": _B_in["x"],
        "B_w1": _B_in["w1"],
        "B_w3": _B_in["w3"],
        "B_w2": _B_in["w2"],
    }

def reference(A_x, A_k_cache, A_v_cache, A_wq, A_wo, B_x, B_w1, B_w3, B_w2):
    def _A_ref(x, k_cache, v_cache, wq, wo):
        B, Sq, D = x.shape
        Hq, Dh = 32, 192
        Hkv, Sk = k_cache.shape[1], k_cache.shape[2]
        W = min(4096, max(256, Sk // 4))
        rep = Hq // Hkv
        q = (lambda x, *d: x.transpose(*d))((x @ wq).reshape(B, Sq, Hq, Dh), 0, 2, 1, 3)
        k = jnp.repeat(k_cache[:, :, Sk - W:, :], rep, axis=1)
        v = jnp.repeat(v_cache[:, :, Sk - W:, :], rep, axis=1)
        scores = jnp.einsum("bhqd,bhkd->bhqk", q, k) * (Dh ** -0.5)
        p = _softmax(scores, axis=-1)
        o = jnp.einsum("bhqk,bhkd->bhqd", p, v)
        return (lambda x, *d: x.transpose(*d))(o, 0, 2, 1, 3).reshape(B, Sq, Hq * Dh) @ wo

    def _B_ref(x, w1, w3, w2):
        gate = jnp.einsum("bsd,df->bsf", x, w1)
        up = jnp.einsum("bsd,df->bsf", x, w3)
        h = _silu(gate) * up
        out = jnp.einsum("bsf,fd->bsd", h, w2)
        return out

    x = A_x
    h = x + _A_ref(_layernorm(x, axis=-1), A_k_cache, A_v_cache, A_wq, A_wo)
    h2 = h + _B_ref(_layernorm(h, axis=-1), B_w1, B_w3, B_w2)
    return h2
```

```python
import re

import jax
import jax.numpy as jnp
import numpy as np
from jax import lax
import jax.experimental.pallas as pl
import jax.experimental.pallas.tpu as pltpu

H, DH, SK, D, F = 32, 192, 32768, 640, 1536
W = min(4096, max(256, SK // 4))
BF = jnp.bfloat16
F32 = jnp.float32


def _bf16_round(v):
    u = int(np.float32(v).view(np.uint32))
    u = (u + 0x7FFF + ((u >> 16) & 1)) & 0xFFFF0000
    return float(np.uint32(u).view(np.float32))


SCALE = _bf16_round(DH ** -0.5)
EPS = _bf16_round(1e-5)


def _r(x):
    return x.astype(BF).astype(F32)


def _layernorm(x32):
    m = jnp.mean(x32, axis=-1, keepdims=True)
    c = x32 - m
    v = jnp.mean(c * c, axis=-1, keepdims=True)
    num = _r(x32 - _r(m))
    den = _r(jnp.sqrt(_r(_r(v) + EPS)))
    return (num / den).astype(BF)


RUN = 512
GF, MF = 15, 64
GW = 4


def _parts(sizes):
    return [(sum(sizes[:i]), n) for i, n in enumerate(sizes)]


def _merge(a, b):
    out, ia, ib = [], 0, 0
    while ia < len(a) or ib < len(b):
        if ib >= len(b) or (ia < len(a) and ia * len(b) <= ib * len(a)):
            out.append(a[ia])
            ia += 1
        else:
            out.append(b[ib])
            ib += 1
    return out


def _split(lst, n):
    return [lst[i * len(lst) // n:(i + 1) * len(lst) // n] for i in range(n)]


def _runs(w):
    rows, cols = w.shape
    t = w.reshape(rows // 8, 8, cols // 128, 128).transpose(0, 2, 1, 3)
    t = t.reshape(-1, RUN // 128, 8, 128).transpose(0, 2, 1, 3)
    return t.reshape(GF, MF, 8, RUN)


def make_kernel(R=3, kpart=(5, 5, 5, 5, 4), vpart=(5, 5, 5, 5, 4), kcols=(0, 1, 2, 3, 4, 5, 6, 7), vcols=(0, 1, 2, 3, 4, 5, 6, 7),
                qpart=(5, 4, 3, 3), opart=(5, 4, 3, 3), first=(), nf=1, n0=60,
                w2ch="128m216 128m216 64m216 48v216 16v28", sh=0,
                tail_split=(25, 60, 120), nocheck=False):
    NQ = 4
    QC = H // NQ
    w2ch = [(int(a), k, int(b[0]), int(b[1:]), cy or "01") for a, k, b, cy in re.findall(r"(\d+)([mv])(\d+):?(\d*)", w2ch)]
    N2 = len(w2ch)
    RW1, RW2 = D // GW, F // GW
    w2off = [sum(c[0] for c in w2ch[:i]) for i in range(N2)]
    assert sum(c[0] for c in w2ch) == RW2

    def grid_pieces(part):
        return [((g, n), (m, 1)) for m in range(MF) for g, n in _parts(first[m] if m < len(first) else part)]

    def kv_pieces(part, cols):
        return [((8 * r, 8 * n), (c * RUN, RUN)) for c in cols for r, n in _parts(part)]

    def kernel(x_hbm, kt_hbm, vt_hbm, wq_hbm, wo_hbm, w1_hbm, w3_hbm, w2_hbm, o_hbm,
               x_v, wq_v, q_v, kbuf, vbuf, wo_v, w13_v, w2_v, o_v, sem_o):

        def body(sem_x, sem_f, sem_wq, sem_k, sem_v, sem_wo, sem_w13, sem_w2):
            def issue(jobs):
                for (src, dst, sem, p, thread) in jobs:
                    idx = tuple(pl.ds(*s) for s in p)
                    pltpu.make_async_copy(src.at[idx], dst.at[idx], sem).start(priority=thread)

            def wait_all(ref, sem):
                pltpu.make_async_copy(ref, ref, sem).wait()

            def head_jobs(h, slot):
                ksrc = kt_hbm.at[h, :, pl.ds(SK - W, W)]
                vsrc = vt_hbm.at[h, :, pl.ds(SK - W, W)]
                return _merge([(ksrc, kbuf.at[slot], sem_k.at[slot], p, 0) for p in kv_pieces(kpart, kcols)],
                              [(vsrc, vbuf.at[slot], sem_v.at[slot], p, 1) for p in kv_pieces(vpart, vcols)])

            x_copy = pltpu.make_async_copy(x_hbm, x_v, sem_x)
            x_copy.start()
            issue(_merge([(wq_hbm, wq_v, sem_f if p[1][0] < nf else sem_wq, p, 0) for p in grid_pieces(qpart)],
                         [(wo_hbm, wo_v, sem_wo.at[p[1][0] * NQ // MF], p, 1) for p in grid_pieces(opart)]))
            wait_all(wq_v.at[:, pl.ds(0, nf)], sem_f)
            jobs = []
            for h in range(R):
                jobs += head_jobs(h, h)
            issue(jobs[:n0])

            x_copy.wait()
            x32 = x_v[...].astype(F32)
            lnx = jnp.broadcast_to(_layernorm(x32), (8, D))
            wait_all(wq_v.at[:, pl.ds(nf, MF - nf)], sem_wq)
            JB = H * DH // RUN
            groups = _split(jobs[n0:], NQ + 1)
            for c in range(NQ):
                wait_all(wo_v.at[:, pl.ds(c * MF // NQ, MF // NQ)], sem_wo.at[c])
                issue(groups[c])
                qc = []
                for j in range(c * JB // NQ, (c + 1) * JB // NQ):
                    rhs = jnp.concatenate([wq_v[divmod(r * JB + j, MF)] for r in range(D // 8)], axis=0)
                    qc.append(jnp.dot(lnx, rhs, preferred_element_type=F32))
                qc = jnp.concatenate(qc, axis=1)
                for j in range(QC):
                    q_v[c * QC + j] = qc[:, j * DH:(j + 1) * DH]

            def wo_rows(h):
                CB, TR = D // 128, RUN // 128
                nrun = DH // 8 * CB // TR
                runs = []
                for i in range(nrun):
                    k = h * nrun + i
                    runs.append(wo_v[k // MF, k % MF] if isinstance(h, int)
                                else wo_v[lax.shift_right_logical(k, 6), lax.bitwise_and(k, MF - 1)])
                tile = lambda t: runs[t // TR][:, (t % TR) * 128:(t % TR + 1) * 128]
                return jnp.concatenate([jnp.concatenate([tile(r * CB + cb) for r in range(DH // 8)], axis=0)
                                        for cb in range(CB)], axis=1)

            def head_compute(h, slot, attn, after_k=(), after_v=()):
                wait_all(kbuf.at[slot], sem_k.at[slot])
                if not after_v:
                    wait_all(vbuf.at[slot], sem_v.at[slot])
                issue(after_k)
                qh = q_v[h].astype(BF)
                s = jnp.dot(qh, kbuf[slot], preferred_element_type=F32)
                s = _r(_r(s) * SCALE)
                m = jnp.max(s, axis=-1, keepdims=True)
                e = _r(jnp.exp(_r(s - m)))
                l = _r(jnp.sum(e, axis=-1, keepdims=True))
                p = (e / l).astype(BF)
                if after_v:
                    wait_all(vbuf.at[slot], sem_v.at[slot])
                    issue(after_v)
                o = lax.dot_general(p, vbuf[slot], (((1,), (1,)), ((), ())),
                                    preferred_element_type=F32)
                return attn + jnp.dot(o.astype(BF), wo_rows(h), preferred_element_type=F32)

            attn = head_compute(0, 0, jnp.zeros((8, D), F32), groups[NQ])
            issue(head_jobs(R, 0))

            def head(h, attn):
                slot = h % R
                attn = head_compute(h, slot, attn)
                issue(head_jobs(h + R, slot))
                return attn

            attn = lax.fori_loop(1, H - R, head, attn)

            pp = [((0, GW), (r, 8), (c, RUN)) for r in range(0, RW1, 8) for c in range(0, F, RUN)]
            j1 = [(w1_hbm, w13_v.at[0], sem_w13.at[0], p) for p in pp]
            j3 = [(w3_hbm, w13_v.at[1], sem_w13.at[1], p) for p in pp]
            t0, t1 = j1[:len(pp) - sh] + _merge(j1[len(pp) - sh:], j3[len(pp) - sh:]), j3[:len(pp) - sh]
            for c, (nr, _, pg, pr, cyc) in enumerate(w2ch):
                ps = [((g, pg), (w2off[c] + r, min(pr, nr - r))) for r in range(0, nr, pr) for g in range(0, GW, pg)]
                for n, p in enumerate(ps):
                    (t0, t1)[int(cyc[n % len(cyc)])].append((w2_hbm, w2_v, sem_w2.at[c], p))
            jobs = [lst[k] + (t,) for k in range(max(len(t0), len(t1))) for t, lst in enumerate((t0, t1)) if k < len(lst)]
            cuts = ((0,) + tuple(tail_split) + (len(jobs),) * 2)[:R + 3]
            for i, h in enumerate(range(H - R, H)):
                attn = head_compute(h, h % R, attn, jobs[cuts[i]:cuts[i + 1]], jobs[cuts[R]:cuts[R + 1]] if h == H - 1 else ())

            hres = _r(x32 + _r(attn))
            lnh = _layernorm(hres)
            wait_all(w13_v.at[0], sem_w13.at[0])
            issue(jobs[cuts[R + 1]:cuts[R + 2]])
            gate = _r(jnp.dot(lnh, w13_v[0].reshape(D, F), preferred_element_type=F32))
            act = _r(gate * _r(jax.nn.sigmoid(gate)))
            wait_all(w13_v.at[1], sem_w13.at[1])
            issue(jobs[cuts[R + 2]:])
            up = _r(jnp.dot(lnh, w13_v[1].reshape(D, F), preferred_element_type=F32))
            hm32 = _r(act * up)
            hm = hm32.astype(BF)
            hcol = {}
            for c in range(N2):
                if w2ch[c][1] == "v":
                    for g in range(GW):
                        b = (g * RW2 + w2off[c]) // 128
                        if b not in hcol:
                            hcol[b] = jnp.transpose(jnp.broadcast_to(hm32[0:1, b * 128:(b + 1) * 128], (128, 128)))
            out = None
            row0 = lax.broadcasted_iota(jnp.int32, (8, D), 0) == 0
            on_vpu = False
            for c in range(N2):
                r0, nr = w2off[c], w2ch[c][0]
                if w2ch[c][1] == "v" and not on_vpu:
                    out, on_vpu = jnp.where(row0, out, 0.0), True
                wait_all(w2_v.at[:, pl.ds(r0, nr)], sem_w2.at[c])
                for g in range(GW):
                    f0 = g * RW2 + r0
                    if not on_vpu:
                        o_ = jnp.dot(hm[:, f0:f0 + nr], w2_v[g, r0:r0 + nr, :], preferred_element_type=F32)
                        out = o_ if out is None else out + o_
                    else:
                        wv = w2_v[g, r0:r0 + nr, :].astype(F32)
                        for r in range(0, nr, 8):
                            hb = hcol[(f0 + r) // 128][(f0 + r) % 128:(f0 + r) % 128 + 8]
                            out = out + wv[r:r + 8] * jnp.concatenate([hb] * (D // 128), axis=1)
            out = jnp.sum(out, axis=0, keepdims=True) if on_vpu else out[0:1]
            o_v[...] = (hres[0:1] + _r(out)).astype(o_v.dtype)
            pltpu.make_async_copy(o_v, o_hbm, sem_o).start()

        dma = pltpu.SemaphoreType.DMA
        pl.run_scoped(body, dma(()), dma(()), dma(()), dma((R,)), dma((R,)), dma((NQ,)), dma((2,)), dma((N2,)))
        pltpu.make_async_copy(o_v, o_hbm, sem_o).wait()

    @jax.jit
    def run(A_x, A_k_cache, A_v_cache, A_wq, A_wo, B_x, B_w1, B_w3, B_w2):
        del B_x
        x = A_x.reshape(1, D)
        kt = jnp.swapaxes(A_k_cache.reshape(H, SK, DH), 1, 2)
        vt = jnp.swapaxes(A_v_cache.reshape(H, SK, DH), 1, 2)
        out = pl.pallas_call(
            kernel,
            out_shape=jax.ShapeDtypeStruct((1, D), A_x.dtype),
            in_specs=[pl.BlockSpec(memory_space=pl.ANY)] * 8,
            out_specs=pl.BlockSpec(memory_space=pl.ANY),
            scratch_shapes=[
                pltpu.VMEM((1, D), BF),
                pltpu.VMEM((GF, MF, 8, RUN), BF),
                pltpu.VMEM((H, 8, DH), F32),
                pltpu.VMEM((R, DH, W), BF),
                pltpu.VMEM((R, DH, W), BF),
                pltpu.VMEM((GF, MF, 8, RUN), BF),
                pltpu.VMEM((2, GW, RW1, F), BF),
                pltpu.VMEM((GW, RW2, D), BF),
                pltpu.VMEM((1, D), BF),
                pltpu.SemaphoreType.DMA(()),
            ],
            compiler_params=pltpu.CompilerParams(vmem_limit_bytes=64 * 1024 * 1024, disable_bounds_checks=nocheck),
        )(x, kt, vt, _runs(A_wq), _runs(A_wo), B_w1.reshape(GW, RW1, F), B_w3.reshape(GW, RW1, F),
          B_w2.reshape(GW, RW2, D))
        return out.reshape(1, 1, D)

    return run


pallas_sequential_preLN__sliding_block_cached__glu_gated_swiglu__decode_kernel = make_kernel()
```

```python
import re

import jax
import jax.numpy as jnp
import numpy as np
from jax import lax
import jax.experimental.pallas as pl
import jax.experimental.pallas.tpu as pltpu

H, DH, SK, D, F = 32, 192, 32768, 640, 1536
W = min(4096, max(256, SK // 4))
BF = jnp.bfloat16
F32 = jnp.float32


def _bf16_round(v):
    u = int(np.float32(v).view(np.uint32))
    u = (u + 0x7FFF + ((u >> 16) & 1)) & 0xFFFF0000
    return float(np.uint32(u).view(np.float32))


SCALE = _bf16_round(DH ** -0.5)
EPS = _bf16_round(1e-5)


def _r(x):
    return x.astype(BF).astype(F32)


def _layernorm(x32):
    m = jnp.mean(x32, axis=-1, keepdims=True)
    c = x32 - m
    v = jnp.mean(c * c, axis=-1, keepdims=True)
    num = _r(x32 - _r(m))
    den = _r(jnp.sqrt(_r(_r(v) + EPS)))
    return (num / den).astype(BF)


RUN = 512
GF, MF = 15, 64
GW = 4


def _parts(sizes):
    return [(sum(sizes[:i]), n) for i, n in enumerate(sizes)]


def _merge(a, b):
    out, ia, ib = [], 0, 0
    while ia < len(a) or ib < len(b):
        if ib >= len(b) or (ia < len(a) and ia * len(b) <= ib * len(a)):
            out.append(a[ia])
            ia += 1
        else:
            out.append(b[ib])
            ib += 1
    return out


def _split(lst, n):
    return [lst[i * len(lst) // n:(i + 1) * len(lst) // n] for i in range(n)]


def _runs(w):
    rows, cols = w.shape
    t = w.reshape(rows // 8, 8, cols // 128, 128).transpose(0, 2, 1, 3)
    t = t.reshape(-1, RUN // 128, 8, 128).transpose(0, 2, 1, 3)
    return t.reshape(GF, MF, 8, RUN)


def make_kernel(R=2, kpat="5:65445 6:65445 7:65445 4:4453323 1:54447 2:5775 3:53565 0:554325",
                vpat="7:3334533 6:58353 5:58353 4:6765 3:58353 0:3333543 1:4875 2:58353",
                qpart=(5, 4, 3, 3), opart=(5, 4, 3, 3), first="1 1 1 1 2 2 3 3", nf=1, n0=60,
                w2ch="128m216 128m216 64v216 32v28 16v28:1 8v28 8v28",
                tail_split=(40, 120, 150, 160), nocheck=False):
    first = [{1: (1,) * 15, 2: (2, 2, 2, 2, 2, 2, 3), 3: (3, 3, 3, 3, 3)}[int(c)] for c in first.split()]
    NQ = 4
    QC = H // NQ
    w2ch = [(int(a), k, int(b[0]), int(b[1:]), cy or "01") for a, k, b, cy in re.findall(r"(\d+)([mv])(\d+):?(\d*)", w2ch)]
    N2 = len(w2ch)
    RW1, RW2 = D // GW, F // GW
    w2off = [sum(c[0] for c in w2ch[:i]) for i in range(N2)]
    assert sum(c[0] for c in w2ch) == RW2

    def grid_pieces(part):
        return [((g, n), (m, 1)) for m in range(MF) for g, n in _parts(first[m] if m < len(first) else part)]

    def kv_pieces(pat):
        return [((8 * r, 8 * n), (int(col[0]) * RUN, RUN))
                for col in pat.split() for r, n in _parts([int(d) for d in col[2:]])]

    def kernel(x_hbm, kt_hbm, vt_hbm, wq_hbm, wo_hbm, w1_hbm, w3_hbm, w2_hbm, o_hbm,
               x_v, wq_v, q_v, kbuf, vbuf, wo_v, w13_v, w2_v, o_v, sem_o):

        def body(sem_x, sem_f, sem_wq, sem_k, sem_v, sem_wo, sem_w13, sem_w2):
            def issue(jobs):
                for (src, dst, sem, p, thread) in jobs:
                    idx = tuple(pl.ds(*s) for s in p)
                    pltpu.make_async_copy(src.at[idx], dst.at[idx], sem).start(priority=thread)

            def wait_all(ref, sem):
                pltpu.make_async_copy(ref, ref, sem).wait()

            def head_jobs(h, slot):
                ksrc = kt_hbm.at[h, :, pl.ds(SK - W, W)]
                vsrc = vt_hbm.at[h, :, pl.ds(SK - W, W)]
                return _merge([(ksrc, kbuf.at[slot], sem_k.at[slot], p, 0) for p in kv_pieces(kpat)],
                              [(vsrc, vbuf.at[slot], sem_v.at[slot], p, 1) for p in kv_pieces(vpat)])

            x_copy = pltpu.make_async_copy(x_hbm, x_v, sem_x)
            x_copy.start()
            issue(_merge([(wq_hbm, wq_v, sem_f if p[1][0] < nf else sem_wq, p, 0) for p in grid_pieces(qpart)],
                         [(wo_hbm, wo_v, sem_wo.at[p[1][0] * NQ // MF], p, 1) for p in grid_pieces(opart)]))
            wait_all(wq_v.at[:, pl.ds(0, nf)], sem_f)
            jobs = []
            for h in range(R):
                jobs += head_jobs(h, h)
            issue(jobs[:n0])

            x_copy.wait()
            x32 = x_v[...].astype(F32)
            lnx = jnp.broadcast_to(_layernorm(x32), (8, D))
            wait_all(wq_v.at[:, pl.ds(nf, MF - nf)], sem_wq)
            JB = H * DH // RUN
            groups = _split(jobs[n0:], NQ + 1)
            for c in range(NQ):
                wait_all(wo_v.at[:, pl.ds(c * MF // NQ, MF // NQ)], sem_wo.at[c])
                issue(groups[c])
                qc = []
                for j in range(c * JB // NQ, (c + 1) * JB // NQ):
                    rhs = jnp.concatenate([wq_v[divmod(r * JB + j, MF)] for r in range(D // 8)], axis=0)
                    qc.append(jnp.dot(lnx, rhs, preferred_element_type=F32))
                qc = jnp.concatenate(qc, axis=1)
                for j in range(QC):
                    q_v[c * QC + j] = qc[:, j * DH:(j + 1) * DH]

            def wo_rows(h):
                CB, TR = D // 128, RUN // 128
                nrun = DH // 8 * CB // TR
                runs = []
                for i in range(nrun):
                    k = h * nrun + i
                    runs.append(wo_v[k // MF, k % MF] if isinstance(h, int)
                                else wo_v[lax.shift_right_logical(k, 6), lax.bitwise_and(k, MF - 1)])
                tile = lambda t: runs[t // TR][:, (t % TR) * 128:(t % TR + 1) * 128]
                return jnp.concatenate([jnp.concatenate([tile(r * CB + cb) for r in range(DH // 8)], axis=0)
                                        for cb in range(CB)], axis=1)

            def head_compute(h, slot, attn, after_k=(), after_v=()):
                wait_all(kbuf.at[slot], sem_k.at[slot])
                if not after_v:
                    wait_all(vbuf.at[slot], sem_v.at[slot])
                issue(after_k)
                qh = q_v[h].astype(BF)
                s = jnp.dot(qh, kbuf[slot], preferred_element_type=F32)
                s = _r(_r(s) * SCALE)
                m = jnp.max(s, axis=-1, keepdims=True)
                e = _r(jnp.exp(_r(s - m)))
                l = _r(jnp.sum(e, axis=-1, keepdims=True))
                p = (e / l).astype(BF)
                if after_v:
                    wait_all(vbuf.at[slot], sem_v.at[slot])
                    issue(after_v)
                o = lax.dot_general(p, vbuf[slot], (((1,), (1,)), ((), ())),
                                    preferred_element_type=F32)
                return attn + jnp.dot(o.astype(BF), wo_rows(h), preferred_element_type=F32)

            attn = head_compute(0, 0, jnp.zeros((8, D), F32), groups[NQ])
            issue(head_jobs(R, 0))

            def head(h, attn):
                slot = h % R
                attn = head_compute(h, slot, attn)
                issue(head_jobs(h + R, slot))
                return attn

            attn = lax.fori_loop(1, H - R, head, attn)

            pp = [((0, GW), (r, 8), (c, RUN)) for r in range(0, RW1, 8) for c in range(0, F, RUN)]
            j1 = [(w1_hbm, w13_v.at[0], sem_w13.at[0], p) for p in pp]
            j3 = [(w3_hbm, w13_v.at[1], sem_w13.at[1], p) for p in pp]
            t0, t1 = j1, j3
            for c, (nr, _, pg, pr, cyc) in enumerate(w2ch):
                ps = [((g, pg), (w2off[c] + r, min(pr, nr - r))) for r in range(0, nr, pr) for g in range(0, GW, pg)]
                for n, p in enumerate(ps):
                    (t0, t1)[int(cyc[n % len(cyc)])].append((w2_hbm, w2_v, sem_w2.at[c], p))
            jobs = [lst[k] + (t,) for k in range(max(len(t0), len(t1))) for t, lst in enumerate((t0, t1)) if k < len(lst)]
            cuts = ((0,) + tuple(tail_split) + (len(jobs),) * 2)[:R + 3]
            for i, h in enumerate(range(H - R, H)):
                attn = head_compute(h, h % R, attn, jobs[cuts[i]:cuts[i + 1]], jobs[cuts[R]:cuts[R + 1]] if h == H - 1 else ())

            hres = _r(x32 + _r(attn))
            lnh = _layernorm(hres)
            wait_all(w13_v.at[0], sem_w13.at[0])
            issue(jobs[cuts[R + 1]:cuts[R + 2]])
            gate = _r(jnp.dot(lnh, w13_v[0].reshape(D, F), preferred_element_type=F32))
            act = _r(gate * _r(jax.nn.sigmoid(gate)))
            wait_all(w13_v.at[1], sem_w13.at[1])
            issue(jobs[cuts[R + 2]:])
            up = _r(jnp.dot(lnh, w13_v[1].reshape(D, F), preferred_element_type=F32))
            hm32 = _r(act * up)
            hm = hm32.astype(BF)
            hcol = {}
            for c in range(N2):
                if w2ch[c][1] == "v":
                    for g in range(GW):
                      for b in range((g * RW2 + w2off[c]) // 128, (g * RW2 + w2off[c] + w2ch[c][0] - 1) // 128 + 1):
                        if b not in hcol:
                            hcol[b] = jnp.transpose(jnp.broadcast_to(hm32[0:1, b * 128:(b + 1) * 128], (128, 128)))
            out = None
            row0 = lax.broadcasted_iota(jnp.int32, (8, D), 0) == 0
            on_vpu = False
            for c in range(N2):
                r0, nr = w2off[c], w2ch[c][0]
                if w2ch[c][1] == "v" and not on_vpu:
                    out, on_vpu = (jnp.zeros((8, D), F32) if out is None else jnp.where(row0, out, 0.0)), True
                wait_all(w2_v.at[:, pl.ds(r0, nr)], sem_w2.at[c])
                for g in range(GW):
                    f0 = g * RW2 + r0
                    if not on_vpu:
                        o_ = jnp.dot(hm[:, f0:f0 + nr], w2_v[g, r0:r0 + nr, :], preferred_element_type=F32)
                        out = o_ if out is None else out + o_
                    else:
                        wv = w2_v[g, r0:r0 + nr, :].astype(F32)
                        for r in range(0, nr, 8):
                            hb = hcol[(f0 + r) // 128][(f0 + r) % 128:(f0 + r) % 128 + 8]
                            out = out + wv[r:r + 8] * jnp.concatenate([hb] * (D // 128), axis=1)
            out = jnp.sum(out, axis=0, keepdims=True) if on_vpu else out[0:1]
            o_v[...] = (hres[0:1] + _r(out)).astype(o_v.dtype)
            pltpu.make_async_copy(o_v, o_hbm, sem_o).start()

        dma = pltpu.SemaphoreType.DMA
        pl.run_scoped(body, dma(()), dma(()), dma(()), dma((R,)), dma((R,)), dma((NQ,)), dma((2,)), dma((N2,)))
        pltpu.make_async_copy(o_v, o_hbm, sem_o).wait()

    @jax.jit
    def run(A_x, A_k_cache, A_v_cache, A_wq, A_wo, B_x, B_w1, B_w3, B_w2):
        del B_x
        x = A_x.reshape(1, D)
        kt = jnp.swapaxes(A_k_cache.reshape(H, SK, DH), 1, 2)
        vt = jnp.swapaxes(A_v_cache.reshape(H, SK, DH), 1, 2)
        out = pl.pallas_call(
            kernel,
            out_shape=jax.ShapeDtypeStruct((1, D), A_x.dtype),
            in_specs=[pl.BlockSpec(memory_space=pl.ANY)] * 8,
            out_specs=pl.BlockSpec(memory_space=pl.ANY),
            scratch_shapes=[
                pltpu.VMEM((1, D), BF),
                pltpu.VMEM((GF, MF, 8, RUN), BF),
                pltpu.VMEM((H, 8, DH), F32),
                pltpu.VMEM((R, DH, W), BF),
                pltpu.VMEM((R, DH, W), BF),
                pltpu.VMEM((GF, MF, 8, RUN), BF),
                pltpu.VMEM((2, GW, RW1, F), BF),
                pltpu.VMEM((GW, RW2, D), BF),
                pltpu.VMEM((1, D), BF),
                pltpu.SemaphoreType.DMA(()),
            ],
            compiler_params=pltpu.CompilerParams(vmem_limit_bytes=64 * 1024 * 1024, disable_bounds_checks=nocheck),
        )(x, kt, vt, _runs(A_wq), _runs(A_wo), B_w1.reshape(GW, RW1, F), B_w3.reshape(GW, RW1, F),
          B_w2.reshape(GW, RW2, D))
        return out.reshape(1, 1, D)

    return run


pallas_sequential_preLN__sliding_block_cached__glu_gated_swiglu__decode_kernel = make_kernel()
```

```python
import jax
import jax.numpy as jnp
import numpy as np
from jax import lax
import jax.experimental.pallas as pl
import jax.experimental.pallas.tpu as pltpu

H, DH, SK, D, F = 32, 192, 32768, 640, 1536
W = min(4096, max(256, SK // 4))
BF = jnp.bfloat16
F32 = jnp.float32


def _bf16_round(v):
    u = int(np.float32(v).view(np.uint32))
    u = (u + 0x7FFF + ((u >> 16) & 1)) & 0xFFFF0000
    return float(np.uint32(u).view(np.float32))


SCALE = _bf16_round(DH ** -0.5)
EPS = _bf16_round(1e-5)


def _r(x):
    return x.astype(BF).astype(F32)


def _layernorm(x32):
    m = jnp.mean(x32, axis=-1, keepdims=True)
    c = x32 - m
    v = jnp.mean(c * c, axis=-1, keepdims=True)
    num = _r(x32 - _r(m))
    den = _r(jnp.sqrt(_r(_r(v) + EPS)))
    return (num / den).astype(BF)


RUN = 512
GF, MF = 15, 64
GW = 4


def _parts(sizes):
    return [(sum(sizes[:i]), n) for i, n in enumerate(sizes)]


def _merge(a, b):
    out, ia, ib = [], 0, 0
    while ia < len(a) or ib < len(b):
        if ib >= len(b) or (ia < len(a) and ia * len(b) <= ib * len(a)):
            out.append(a[ia])
            ia += 1
        else:
            out.append(b[ib])
            ib += 1
    return out


def _split(lst, n):
    return [lst[i * len(lst) // n:(i + 1) * len(lst) // n] for i in range(n)]


def _runs(w):
    rows, cols = w.shape
    t = w.reshape(rows // 8, 8, cols // 128, 128).transpose(0, 2, 1, 3)
    t = t.reshape(-1, RUN // 128, 8, 128).transpose(0, 2, 1, 3)
    return t.reshape(GF, MF, 8, RUN)


def make_kernel(
        R=2,
        kpat="5:65445 6:65445 7:65445 4:4453323 1:54447 2:5775 3:53565 0:534552",
        vpat="7:4323633 6:43755 5:34575 0:4533234 3:55554 4:6765 1:7755 2:58353",
        qpart=(5, 4, 3, 3), opart=(4, 3, 4, 4),
        ramp=((1,) * 15,) * 4 + ((2, 2, 2, 2, 2, 2, 3),) * 2 + ((3, 3, 3, 3, 3),) * 2,
        w2ch=((128, "M", 2, 16, (0, 1)), (128, "M", 2, 16, (0, 1)), (64, "V", 2, 16, (0, 1)),
              (32, "V", 2, 8, (0, 1)), (16, "V", 2, 8, (1,)), (8, "V", 2, 8, (0, 1)), (8, "V", 2, 8, (0, 1))),
        n0=60,
        tail_split=(40, 120, 150, 160)):
    NQ = 4
    QC = H // NQ
    N2 = len(w2ch)
    RW1, RW2 = D // GW, F // GW
    w2off = [sum(c[0] for c in w2ch[:i]) for i in range(N2)]
    assert sum(c[0] for c in w2ch) == RW2 and len(tail_split) == R + 2

    def grid_pieces(part):
        parts = [ramp[m] if m < len(ramp) else part for m in range(MF)]
        assert all(sum(p) == GF for p in parts)
        return [((g, n), (m, 1)) for m in range(MF) for g, n in _parts(parts[m])]

    def kv_pieces(pat):
        cols = [(int(col[0]), [int(d) for d in col[2:]]) for col in pat.split()]
        assert sorted(c for c, _ in cols) == list(range(W // RUN)) and all(8 * sum(p) == DH for _, p in cols)
        return [((8 * r, 8 * n), (c * RUN, RUN)) for c, p in cols for r, n in _parts(p)]

    def kernel(x_hbm, kt_hbm, vt_hbm, wq_hbm, wo_hbm, w1_hbm, w3_hbm, w2_hbm, o_hbm,
               x_v, wq_v, q_v, kbuf, vbuf, wo_v, w13_v, w2_v, o_v,
               sem_x, sem_f, sem_wq, sem_k, sem_v, sem_wo, sem_w13, sem_w2, sem_o):
        def issue(jobs):
            for (src, dst, sem, p, thread) in jobs:
                idx = tuple(pl.ds(*s) for s in p)
                pltpu.make_async_copy(src.at[idx], dst.at[idx], sem).start(priority=thread)

        def wait_all(ref, sem):
            pltpu.make_async_copy(ref, ref, sem).wait()

        def head_jobs(h, slot):
            ksrc = kt_hbm.at[h, :, pl.ds(SK - W, W)]
            vsrc = vt_hbm.at[h, :, pl.ds(SK - W, W)]
            return _merge([(ksrc, kbuf.at[slot], sem_k.at[slot], p, 0) for p in kv_pieces(kpat)],
                          [(vsrc, vbuf.at[slot], sem_v.at[slot], p, 1) for p in kv_pieces(vpat)])

        x_copy = pltpu.make_async_copy(x_hbm, x_v, sem_x)
        x_copy.start()
        issue(_merge([(wq_hbm, wq_v, sem_f if p[1][0] == 0 else sem_wq, p, 0) for p in grid_pieces(qpart)],
                     [(wo_hbm, wo_v, sem_wo.at[p[1][0] * NQ // MF], p, 1) for p in grid_pieces(opart)]))
        wait_all(wq_v.at[:, pl.ds(0, 1)], sem_f)
        jobs = []
        for h in range(R):
            jobs += head_jobs(h, h)
        issue(jobs[:n0])

        x_copy.wait()
        x32 = x_v[...].astype(F32)
        lnx = jnp.broadcast_to(_layernorm(x32), (8, D))
        wait_all(wq_v.at[:, pl.ds(1, MF - 1)], sem_wq)
        JB = H * DH // RUN
        groups = _split(jobs[n0:], NQ + 1)
        for c in range(NQ):
            wait_all(wo_v.at[:, pl.ds(c * MF // NQ, MF // NQ)], sem_wo.at[c])
            issue(groups[c])
            qc = []
            for j in range(c * JB // NQ, (c + 1) * JB // NQ):
                rhs = jnp.concatenate([wq_v[divmod(r * JB + j, MF)] for r in range(D // 8)], axis=0)
                qc.append(jnp.dot(lnx, rhs, preferred_element_type=F32))
            qc = jnp.concatenate(qc, axis=1)
            for j in range(QC):
                q_v[c * QC + j] = qc[:, j * DH:(j + 1) * DH]

        def wo_rows(h):
            CB, TR = D // 128, RUN // 128
            nrun = DH // 8 * CB // TR
            runs = []
            for i in range(nrun):
                k = h * nrun + i
                runs.append(wo_v[k // MF, k % MF] if isinstance(h, int)
                            else wo_v[lax.shift_right_logical(k, 6), lax.bitwise_and(k, MF - 1)])
            tile = lambda t: runs[t // TR][:, (t % TR) * 128:(t % TR + 1) * 128]
            return jnp.concatenate([jnp.concatenate([tile(r * CB + cb) for r in range(DH // 8)], axis=0)
                                    for cb in range(CB)], axis=1)

        def head_compute(h, slot, attn, after_k=(), after_v=()):
            wait_all(kbuf.at[slot], sem_k.at[slot])
            if not after_v:
                wait_all(vbuf.at[slot], sem_v.at[slot])
            issue(after_k)
            qh = q_v[h].astype(BF)
            s = jnp.dot(qh, kbuf[slot], preferred_element_type=F32)
            s = _r(_r(s) * SCALE)
            m = jnp.max(s, axis=-1, keepdims=True)
            e = _r(jnp.exp(_r(s - m)))
            l = _r(jnp.sum(e, axis=-1, keepdims=True))
            p = (e / l).astype(BF)
            if after_v:
                wait_all(vbuf.at[slot], sem_v.at[slot])
                issue(after_v)
            o = lax.dot_general(p, vbuf[slot], (((1,), (1,)), ((), ())),
                                preferred_element_type=F32)
            return attn + jnp.dot(o.astype(BF), wo_rows(h), preferred_element_type=F32)

        attn = head_compute(0, 0, jnp.zeros((8, D), F32), groups[NQ])
        issue(head_jobs(R, 0))

        def head(h, attn):
            slot = h % R
            attn = head_compute(h, slot, attn)
            issue(head_jobs(h + R, slot))
            return attn

        attn = lax.fori_loop(1, H - R, head, attn)

        pp = [((0, GW), (r, 8), (c, RUN)) for r in range(0, RW1, 8) for c in range(0, F, RUN)]
        t0 = [(w1_hbm, w13_v.at[0], sem_w13.at[0], p) for p in pp]
        t1 = [(w3_hbm, w13_v.at[1], sem_w13.at[1], p) for p in pp]
        for c, (nr, _, pg, pr, cyc) in enumerate(w2ch):
            ps = [((g, pg), (w2off[c] + r, min(pr, nr - r))) for r in range(0, nr, pr) for g in range(0, GW, pg)]
            for n, p in enumerate(ps):
                (t0, t1)[cyc[n % len(cyc)]].append((w2_hbm, w2_v, sem_w2.at[c], p))
        jobs = [lst[k] + (t,) for k in range(max(len(t0), len(t1))) for t, lst in enumerate((t0, t1)) if k < len(lst)]
        cuts = (0,) + tuple(tail_split) + (len(jobs),)
        for i, h in enumerate(range(H - R, H)):
            attn = head_compute(h, h % R, attn, jobs[cuts[i]:cuts[i + 1]], jobs[cuts[R]:cuts[R + 1]] if h == H - 1 else ())

        hres = _r(x32 + _r(attn))
        lnh = _layernorm(hres)
        wait_all(w13_v.at[0], sem_w13.at[0])
        issue(jobs[cuts[R + 1]:cuts[R + 2]])
        gate = _r(jnp.dot(lnh, w13_v[0].reshape(D, F), preferred_element_type=F32))
        act = _r(gate * _r(jax.nn.sigmoid(gate)))
        wait_all(w13_v.at[1], sem_w13.at[1])
        issue(jobs[cuts[R + 2]:])
        up = _r(jnp.dot(lnh, w13_v[1].reshape(D, F), preferred_element_type=F32))
        hm32 = _r(act * up)
        hm = hm32.astype(BF)
        hcol = {}
        for c in range(N2):
            for g in range(GW if w2ch[c][1] == "V" else 0):
                f0 = g * RW2 + w2off[c]
                for b in range(f0 // 128, (f0 + w2ch[c][0] - 1) // 128 + 1):
                    if b not in hcol:
                        hcol[b] = jnp.transpose(jnp.broadcast_to(hm32[0:1, b * 128:(b + 1) * 128], (128, 128)))
        out = None
        row0 = lax.broadcasted_iota(jnp.int32, (8, D), 0) == 0
        on_vpu = False
        for c in range(N2):
            r0, nr = w2off[c], w2ch[c][0]
            if w2ch[c][1] == "V" and not on_vpu:
                out, on_vpu = (jnp.zeros((8, D), F32) if out is None else jnp.where(row0, out, 0.0)), True
            wait_all(w2_v.at[:, pl.ds(r0, nr)], sem_w2.at[c])
            for g in range(GW):
                f0 = g * RW2 + r0
                if not on_vpu:
                    o_ = jnp.dot(hm[:, f0:f0 + nr], w2_v[g, r0:r0 + nr, :], preferred_element_type=F32)
                    out = o_ if out is None else out + o_
                else:
                    wv = w2_v[g, r0:r0 + nr, :].astype(F32)
                    for r in range(0, nr, 8):
                        hb = hcol[(f0 + r) // 128][(f0 + r) % 128:(f0 + r) % 128 + 8]
                        out = out + wv[r:r + 8] * jnp.concatenate([hb] * (D // 128), axis=1)
        out = jnp.sum(out, axis=0, keepdims=True) if on_vpu else out[0:1]
        o_v[...] = (hres[0:1] + _r(out)).astype(o_v.dtype)
        out_copy = pltpu.make_async_copy(o_v, o_hbm, sem_o)
        out_copy.start()
        out_copy.wait()

    @jax.jit
    def run(A_x, A_k_cache, A_v_cache, A_wq, A_wo, B_x, B_w1, B_w3, B_w2):
        del B_x
        x = A_x.reshape(1, D)
        kt = jnp.swapaxes(A_k_cache.reshape(H, SK, DH), 1, 2)
        vt = jnp.swapaxes(A_v_cache.reshape(H, SK, DH), 1, 2)
        dma = pltpu.SemaphoreType.DMA
        out = pl.pallas_call(
            kernel,
            out_shape=jax.ShapeDtypeStruct((1, D), A_x.dtype),
            in_specs=[pl.BlockSpec(memory_space=pl.ANY)] * 8,
            out_specs=pl.BlockSpec(memory_space=pl.ANY),
            scratch_shapes=[
                pltpu.VMEM((1, D), BF),
                pltpu.VMEM((GF, MF, 8, RUN), BF),
                pltpu.VMEM((H, 8, DH), F32),
                pltpu.VMEM((R, DH, W), BF),
                pltpu.VMEM((R, DH, W), BF),
                pltpu.VMEM((GF, MF, 8, RUN), BF),
                pltpu.VMEM((2, GW, RW1, F), BF),
                pltpu.VMEM((GW, RW2, D), BF),
                pltpu.VMEM((1, D), BF),
                dma(()), dma(()), dma(()), dma((R,)), dma((R,)), dma((NQ,)), dma((2,)), dma((N2,)), dma(()),
            ],
            compiler_params=pltpu.CompilerParams(vmem_limit_bytes=64 * 1024 * 1024, disable_semaphore_checks=True),
        )(x, kt, vt, _runs(A_wq), _runs(A_wo), B_w1.reshape(GW, RW1, F), B_w3.reshape(GW, RW1, F),
          B_w2.reshape(GW, RW2, D))
        return out.reshape(1, 1, D)

    return run


pallas_sequential_preLN__sliding_block_cached__glu_gated_swiglu__decode_kernel = make_kernel()
```

```python
import jax
import jax.numpy as jnp
import numpy as np
from jax import lax
import jax.experimental.pallas as pl
import jax.experimental.pallas.tpu as pltpu

H, DH, SK, D, F = 32, 192, 32768, 640, 1536
W = min(4096, max(256, SK // 4))
BF = jnp.bfloat16
F32 = jnp.float32


def _bf16_round(v):
    u = int(np.float32(v).view(np.uint32))
    u = (u + 0x7FFF + ((u >> 16) & 1)) & 0xFFFF0000
    return float(np.uint32(u).view(np.float32))


SCALE = _bf16_round(DH ** -0.5)
EPS = _bf16_round(1e-5)


def _r(x):
    return x.astype(BF).astype(F32)


def _layernorm(x32):
    m = jnp.mean(x32, axis=-1, keepdims=True)
    c = x32 - m
    v = jnp.mean(c * c, axis=-1, keepdims=True)
    num = _r(x32 - _r(m))
    den = _r(jnp.sqrt(_r(_r(v) + EPS)))
    return (num / den).astype(BF)


RUN = 512
GF, MF = 15, 64
GW = 4


def _parts(sizes):
    return [(sum(sizes[:i]), n) for i, n in enumerate(sizes)]


def _merge(a, b):
    out, ia, ib = [], 0, 0
    while ia < len(a) or ib < len(b):
        if ib >= len(b) or (ia < len(a) and ia * len(b) <= ib * len(a)):
            out.append(a[ia])
            ia += 1
        else:
            out.append(b[ib])
            ib += 1
    return out


def _split(lst, n):
    return [lst[i * len(lst) // n:(i + 1) * len(lst) // n] for i in range(n)]


def _runs(w):
    rows, cols = w.shape
    t = w.reshape(rows // 8, 8, cols // 128, 128).transpose(0, 2, 1, 3)
    t = t.reshape(-1, RUN // 128, 8, 128).transpose(0, 2, 1, 3)
    return t.reshape(GF, MF, 8, RUN)


def make_kernel(
        R=2,
        kpat="5:65445 6:65445 7:65445 4:4453323 1:54447 2:5775 3:53565 0:534552",
        vpat="7:4323633 6:43755 5:34575 0:4533234 3:55554 4:6765 1:7755 2:58353",
        qpart=(5, 4, 3, 3), opart=(4, 3, 4, 4),
        ramp=((1,) * 15,) * 4 + ((2, 2, 2, 2, 2, 2, 3),) * 2 + ((3, 3, 3, 3, 3),) * 2,
        w2ch=((128, "M", 2, 16, (0, 1)), (128, "M", 2, 16, (0, 1)), (64, "V", 2, 16, (0, 1)),
              (32, "V", 2, 8, (0, 1)), (16, "V", 2, 8, (1,)), (8, "V", 2, 8, (0, 1)), (8, "V", 2, 8, (0, 1))),
        n0=60,
        tail_split=(40, 120, 150, 160)):
    NQ = 4
    QC = H // NQ
    N2 = len(w2ch)
    RW1, RW2 = D // GW, F // GW
    w2off = [sum(c[0] for c in w2ch[:i]) for i in range(N2)]
    assert sum(c[0] for c in w2ch) == RW2 and len(tail_split) == R + 2

    def grid_pieces(part):
        parts = [ramp[m] if m < len(ramp) else part for m in range(MF)]
        assert all(sum(p) == GF for p in parts)
        return [((g, n), (m, 1)) for m in range(MF) for g, n in _parts(parts[m])]

    def kv_pieces(pat):
        cols = [(int(col[0]), [int(d) for d in col[2:]]) for col in pat.split()]
        assert sorted(c for c, _ in cols) == list(range(W // RUN)) and all(8 * sum(p) == DH for _, p in cols)
        return [((8 * r, 8 * n), (c * RUN, RUN)) for c, p in cols for r, n in _parts(p)]

    def kernel(x_hbm, kt_hbm, vt_hbm, wq_hbm, wo_hbm, w1_hbm, w3_hbm, w2_hbm, o_hbm,
               x_v, wq_v, q_v, kbuf, vbuf, wo_v, w13_v, w2_v, o_v, sem_o):

        def body(sem_x, sem_f, sem_wq, sem_k, sem_v, sem_wo, sem_w13, sem_w2):
            def issue(jobs):
                for (src, dst, sem, p, thread) in jobs:
                    idx = tuple(pl.ds(*s) for s in p)
                    pltpu.make_async_copy(src.at[idx], dst.at[idx], sem).start(priority=thread)

            def wait_all(ref, sem):
                pltpu.make_async_copy(ref, ref, sem).wait()

            def head_jobs(h, slot):
                ksrc = kt_hbm.at[h, :, pl.ds(SK - W, W)]
                vsrc = vt_hbm.at[h, :, pl.ds(SK - W, W)]
                return _merge([(ksrc, kbuf.at[slot], sem_k.at[slot], p, 0) for p in kv_pieces(kpat)],
                              [(vsrc, vbuf.at[slot], sem_v.at[slot], p, 1) for p in kv_pieces(vpat)])

            x_copy = pltpu.make_async_copy(x_hbm, x_v, sem_x)
            x_copy.start()
            issue(_merge([(wq_hbm, wq_v, sem_f if p[1][0] == 0 else sem_wq, p, 0) for p in grid_pieces(qpart)],
                         [(wo_hbm, wo_v, sem_wo.at[p[1][0] * NQ // MF], p, 1) for p in grid_pieces(opart)]))
            wait_all(wq_v.at[:, pl.ds(0, 1)], sem_f)
            jobs = []
            for h in range(R):
                jobs += head_jobs(h, h)
            issue(jobs[:n0])

            x_copy.wait()
            x32 = x_v[...].astype(F32)
            lnx = jnp.broadcast_to(_layernorm(x32), (8, D))
            wait_all(wq_v.at[:, pl.ds(1, MF - 1)], sem_wq)
            JB = H * DH // RUN
            groups = _split(jobs[n0:], NQ + 1)
            for c in range(NQ):
                wait_all(wo_v.at[:, pl.ds(c * MF // NQ, MF // NQ)], sem_wo.at[c])
                issue(groups[c])
                qc = []
                for j in range(c * JB // NQ, (c + 1) * JB // NQ):
                    rhs = jnp.concatenate([wq_v[divmod(r * JB + j, MF)] for r in range(D // 8)], axis=0)
                    qc.append(jnp.dot(lnx, rhs, preferred_element_type=F32))
                qc = jnp.concatenate(qc, axis=1)
                for j in range(QC):
                    q_v[c * QC + j] = qc[:, j * DH:(j + 1) * DH]

            def wo_rows(h):
                CB, TR = D // 128, RUN // 128
                nrun = DH // 8 * CB // TR
                runs = []
                for i in range(nrun):
                    k = h * nrun + i
                    runs.append(wo_v[k // MF, k % MF] if isinstance(h, int)
                                else wo_v[lax.shift_right_logical(k, 6), lax.bitwise_and(k, MF - 1)])
                tile = lambda t: runs[t // TR][:, (t % TR) * 128:(t % TR + 1) * 128]
                return jnp.concatenate([jnp.concatenate([tile(r * CB + cb) for r in range(DH // 8)], axis=0)
                                        for cb in range(CB)], axis=1)

            def head_compute(h, slot, attn, after_k=(), after_v=()):
                wait_all(kbuf.at[slot], sem_k.at[slot])
                if not after_v:
                    wait_all(vbuf.at[slot], sem_v.at[slot])
                issue(after_k)
                qh = q_v[h].astype(BF)
                s = jnp.dot(qh, kbuf[slot], preferred_element_type=F32)
                s = _r(_r(s) * SCALE)
                m = jnp.max(s, axis=-1, keepdims=True)
                e = _r(jnp.exp(_r(s - m)))
                l = _r(jnp.sum(e, axis=-1, keepdims=True))
                p = (e / l).astype(BF)
                if after_v:
                    wait_all(vbuf.at[slot], sem_v.at[slot])
                    issue(after_v)
                o = lax.dot_general(p, vbuf[slot], (((1,), (1,)), ((), ())),
                                    preferred_element_type=F32)
                return attn + jnp.dot(o.astype(BF), wo_rows(h), preferred_element_type=F32)

            attn = head_compute(0, 0, jnp.zeros((8, D), F32), groups[NQ])
            issue(head_jobs(R, 0))

            def head(h, attn):
                slot = h % R
                attn = head_compute(h, slot, attn)
                issue(head_jobs(h + R, slot))
                return attn

            attn = lax.fori_loop(1, H - R, head, attn)

            pp = [((0, GW), (r, 8), (c, RUN)) for r in range(0, RW1, 8) for c in range(0, F, RUN)]
            t0 = [(w1_hbm, w13_v.at[0], sem_w13.at[0], p) for p in pp]
            t1 = [(w3_hbm, w13_v.at[1], sem_w13.at[1], p) for p in pp[1:] + pp[:1]]
            for c, (nr, _, pg, pr, cyc) in enumerate(w2ch):
                ps = [((g, pg), (w2off[c] + r, min(pr, nr - r))) for r in range(0, nr, pr) for g in range(0, GW, pg)]
                for n, p in enumerate(ps):
                    (t0, t1)[cyc[n % len(cyc)]].append((w2_hbm, w2_v, sem_w2.at[c], p))
            jobs = [lst[k] + (t,) for k in range(max(len(t0), len(t1))) for t, lst in enumerate((t0, t1)) if k < len(lst)]
            cuts = (0,) + tuple(tail_split) + (len(jobs),)
            for i, h in enumerate(range(H - R, H)):
                attn = head_compute(h, h % R, attn, jobs[cuts[i]:cuts[i + 1]], jobs[cuts[R]:cuts[R + 1]] if h == H - 1 else ())

            hres = _r(x32 + _r(attn))
            lnh = _layernorm(hres)
            wait_all(w13_v.at[0], sem_w13.at[0])
            issue(jobs[cuts[R + 1]:cuts[R + 2]])
            gate = _r(jnp.dot(lnh, w13_v[0].reshape(D, F), preferred_element_type=F32))
            act = _r(gate * _r(jax.nn.sigmoid(gate)))
            wait_all(w13_v.at[1], sem_w13.at[1])
            issue(jobs[cuts[R + 2]:])
            up = _r(jnp.dot(lnh, w13_v[1].reshape(D, F), preferred_element_type=F32))
            hm32 = _r(act * up)
            hm = hm32.astype(BF)
            hcol = {}
            for c in range(N2):
                for g in range(GW if w2ch[c][1] == "V" else 0):
                    f0 = g * RW2 + w2off[c]
                    for b in range(f0 // 128, (f0 + w2ch[c][0] - 1) // 128 + 1):
                        if b not in hcol:
                            hcol[b] = jnp.transpose(jnp.broadcast_to(hm32[0:1, b * 128:(b + 1) * 128], (128, 128)))
            out = None
            row0 = lax.broadcasted_iota(jnp.int32, (8, D), 0) == 0
            on_vpu = False
            for c in range(N2):
                r0, nr = w2off[c], w2ch[c][0]
                if w2ch[c][1] == "V" and not on_vpu:
                    out, on_vpu = (jnp.zeros((8, D), F32) if out is None else jnp.where(row0, out, 0.0)), True
                wait_all(w2_v.at[:, pl.ds(r0, nr)], sem_w2.at[c])
                for g in range(GW):
                    f0 = g * RW2 + r0
                    if not on_vpu:
                        o_ = jnp.dot(hm[:, f0:f0 + nr], w2_v[g, r0:r0 + nr, :], preferred_element_type=F32)
                        out = o_ if out is None else out + o_
                    else:
                        wv = w2_v[g, r0:r0 + nr, :].astype(F32)
                        for r in range(0, nr, 8):
                            hb = hcol[(f0 + r) // 128][(f0 + r) % 128:(f0 + r) % 128 + 8]
                            out = out + wv[r:r + 8] * jnp.concatenate([hb] * (D // 128), axis=1)
            out = jnp.sum(out, axis=0, keepdims=True) if on_vpu else out[0:1]
            o_v[...] = (hres[0:1] + _r(out)).astype(o_v.dtype)
            pltpu.make_async_copy(o_v, o_hbm, sem_o).start()

        dma = pltpu.SemaphoreType.DMA
        pl.run_scoped(body, dma(()), dma(()), dma(()), dma((R,)), dma((R,)), dma((NQ,)), dma((2,)), dma((N2,)))
        pltpu.make_async_copy(o_v, o_hbm, sem_o).wait()

    @jax.jit
    def run(A_x, A_k_cache, A_v_cache, A_wq, A_wo, B_x, B_w1, B_w3, B_w2):
        del B_x
        x = A_x.reshape(1, D)
        kt = jnp.swapaxes(A_k_cache.reshape(H, SK, DH), 1, 2)
        vt = jnp.swapaxes(A_v_cache.reshape(H, SK, DH), 1, 2)
        out = pl.pallas_call(
            kernel,
            out_shape=jax.ShapeDtypeStruct((1, D), A_x.dtype),
            in_specs=[pl.BlockSpec(memory_space=pl.ANY)] * 8,
            out_specs=pl.BlockSpec(memory_space=pl.ANY),
            scratch_shapes=[
                pltpu.VMEM((1, D), BF),
                pltpu.VMEM((GF, MF, 8, RUN), BF),
                pltpu.VMEM((H, 8, DH), F32),
                pltpu.VMEM((R, DH, W), BF),
                pltpu.VMEM((R, DH, W), BF),
                pltpu.VMEM((GF, MF, 8, RUN), BF),
                pltpu.VMEM((2, GW, RW1, F), BF),
                pltpu.VMEM((GW, RW2, D), BF),
                pltpu.VMEM((1, D), BF),
                pltpu.SemaphoreType.DMA(()),
            ],
            compiler_params=pltpu.CompilerParams(vmem_limit_bytes=64 * 1024 * 1024),
        )(x, kt, vt, _runs(A_wq), _runs(A_wo), B_w1.reshape(GW, RW1, F), B_w3.reshape(GW, RW1, F),
          B_w2.reshape(GW, RW2, D))
        return out.reshape(1, 1, D)

    return run


pallas_sequential_preLN__sliding_block_cached__glu_gated_swiglu__decode_kernel = make_kernel()
```
